```python
import os as _os
_os.environ.setdefault("JAX_PLATFORMS", "cpu")
import jax
import jax.numpy as jnp

def _softmax(x, axis=-1):
    return jax.nn.softmax(x, axis=axis)
def _gelu(x):
    return jax.nn.gelu(x, approximate=True)
def _silu(x):
    return jax.nn.silu(x)
def _sigmoid(x):
    return jax.nn.sigmoid(x)
def _layernorm(x, axis=-1, eps=1e-5):
    m = jnp.mean(x, axis=axis, keepdims=True)
    v = jnp.var(x, axis=axis, keepdims=True)
    return (x - m) / jnp.sqrt(v + eps)
def _scatter_add(tgt, idx, src, axis=0):
    return tgt.at[idx].add(src)
def _segment_sum(src, seg, n):
    return jax.ops.segment_sum(src, seg, n)
class _Rng:
    def __init__(self, key):
        self._k = key
    def _next(self):
        self._k, sub = jax.random.split(self._k)
        return sub
    def normal(self, shape):
        return jax.random.normal(self._next(), shape, dtype=jnp.bfloat16)
    def randint(self, lo, hi, shape):
        return jax.random.randint(self._next(), shape, lo, hi, dtype=jnp.int32)
    def uniform(self, shape, lo=0.0, hi=1.0):
        return jax.random.uniform(self._next(), shape, jnp.bfloat16, lo, hi)
    def permutation(self, n):
        return jax.random.permutation(self._next(), n)


kernel_name = 'standalone__instancenorm__sampling'

def setup_inputs():
    _rng = _Rng(jax.random.key(int.from_bytes(__import__("os").urandom(4), "little")))
    _w = (lambda a: (lambda t: t.astype(jnp.bfloat16) if jnp.issubdtype(t.dtype, jnp.floating) else t)(jnp.asarray(a)))
    B, C, H, W = 16, 640, 16, 32
    return {
        "x": _w((lambda *s: _rng.normal(s) * 0.05)(B, C, H, W)),
        "g": _w((lambda *s: _rng.normal(s) * 0.05)(C) + 1.0),
        "b": _w((lambda *s: _rng.normal(s) * 0.05)(C)),
    }

def reference(x, g, b):
    mu = x.mean(axis=(-2, -1), keepdims=True)
    var = ((x - mu) * (x - mu)).mean(axis=(-2, -1), keepdims=True)
    xhat = (x - mu) / jnp.sqrt(var + 1e-5)
    return xhat * g.reshape(1, -1, 1, 1) + b.reshape(1, -1, 1, 1)
```

```python
import functools

import jax
import jax.numpy as jnp
import jax.experimental.pallas as pl
import jax.experimental.pallas.tpu as pltpu

_EPS = 1e-5
_ROWS = 8
_NACC = 2


def _normalize_instance(xbuf, bi, g, b):
    _, HW, _ = xbuf.shape
    inv_n = 1.0 / HW

    def tile(r):
        return xbuf[bi, pl.ds(r, _ROWS), :].astype(jnp.float32)

    def row_sum(fn):
        acc = [None] * _NACC
        for k, r in enumerate(range(0, HW, _ROWS)):
            v = fn(tile(r))
            acc[k % _NACC] = v if acc[k % _NACC] is None else acc[k % _NACC] + v
        s = functools.reduce(lambda p, q: p + q, acc)
        return jnp.sum(s, axis=0, keepdims=True)

    mu = row_sum(lambda t: t) * inv_n

    def sq(t):
        d = t - mu
        return d * d

    var = row_sum(sq) * inv_n
    scale = jax.lax.rsqrt(var + _EPS) * g
    for r in range(0, HW, _ROWS):
        xbuf[bi, pl.ds(r, _ROWS), :] = ((tile(r) - mu) * scale + b).astype(xbuf.dtype)


def _kernel(x_hbm, g_hbm, b_hbm, o_hbm, xbuf, gbuf, bbuf, sems, gsem, *, rb, wb, wtrig):
    B, HW, C = xbuf.shape
    nr, nw = len(rb) - 1, len(wb) - 1

    def rd(k):
        n = rb[k + 1] - rb[k]
        return pltpu.make_async_copy(
            x_hbm.at[pl.ds(rb[k], n)], xbuf.at[pl.ds(rb[k], n)], sems.at[k])

    def wr(k):
        n = wb[k + 1] - wb[k]
        return pltpu.make_async_copy(
            xbuf.at[pl.ds(wb[k], n)], o_hbm.at[pl.ds(wb[k], n)], sems.at[nr + k])

    gc = pltpu.make_async_copy(g_hbm, gbuf, gsem.at[0])
    bc = pltpu.make_async_copy(b_hbm, bbuf, gsem.at[1])
    gc.start()
    bc.start()

    def issue(i, carry):
        for k in range(nr):
            @pl.when(i == k)
            def _():
                rd(k).start()
        return carry

    jax.lax.fori_loop(0, nr, issue, 0)
    gc.wait()
    bc.wait()
    g = gbuf[...].astype(jnp.float32).reshape(1, C)
    b = bbuf[...].astype(jnp.float32).reshape(1, C)

    def body(bi, carry):
        for k in range(nr):
            @pl.when(bi == rb[k])
            def _():
                rd(k).wait()
        for j in range(nw):
            if wtrig[j] < B:
                @pl.when(bi == wtrig[j])
                def _():
                    wr(j).start()
        _normalize_instance(xbuf, bi, g, b)
        return carry

    jax.lax.fori_loop(0, B, body, 0)
    for j in range(nw):
        if wtrig[j] >= B:
            wr(j).start()
    for j in range(nw):
        wr(j).wait()


@jax.jit
def pallas_standalone__instancenorm__sampling_kernel(
    x: jax.Array,
    g: jax.Array,
    b: jax.Array,
):
    B, C, H, W = x.shape
    HW = H * W
    xt = jnp.transpose(x, (0, 2, 3, 1)).reshape(B, HW, C)

    rb = (0, B // 2, B - 1, B)
    wb = (0, B // 2, B)
    wtrig = (B // 2, B)

    out = pl.pallas_call(
        functools.partial(_kernel, rb=rb, wb=wb, wtrig=wtrig),
        in_specs=[pl.BlockSpec(memory_space=pl.ANY)] * 3,
        out_specs=pl.BlockSpec(memory_space=pl.ANY),
        out_shape=jax.ShapeDtypeStruct((B, HW, C), x.dtype),
        scratch_shapes=[
            pltpu.VMEM((B, HW, C), x.dtype),
            pltpu.VMEM((C,), g.dtype),
            pltpu.VMEM((C,), b.dtype),
            pltpu.SemaphoreType.DMA((len(rb) + len(wb) - 2,)),
            pltpu.SemaphoreType.DMA((2,)),
        ],
        compiler_params=pltpu.CompilerParams(vmem_limit_bytes=48 * 1024 * 1024),
    )(xt, g, b)
    return jnp.transpose(out.reshape(B, H, W, C), (0, 3, 1, 2))
```

```python
import functools

import jax
import jax.numpy as jnp
import jax.experimental.pallas as pl
import jax.experimental.pallas.tpu as pltpu

_EPS = 1e-5
_ROWS = 8
_NACC = 2


def _normalize_instance(xs, g, b):
    HW, _ = xs.shape
    inv_n = 1.0 / HW

    def tile(r):
        return xs[pl.ds(r, _ROWS), :].astype(jnp.float32)

    def column_sum(fn):
        acc = [None] * _NACC
        for k, r in enumerate(range(0, HW, _ROWS)):
            v = fn(tile(r))
            acc[k % _NACC] = v if acc[k % _NACC] is None else acc[k % _NACC] + v
        total = functools.reduce(lambda p, q: p + q, acc)
        return jnp.sum(total, axis=0, keepdims=True)

    mu = column_sum(lambda t: t) * inv_n

    def centered_sq(t):
        d = t - mu
        return d * d

    var = column_sum(centered_sq) * inv_n
    scale = jax.lax.rsqrt(var + _EPS) * g
    for r in range(0, HW, _ROWS):
        xs[pl.ds(r, _ROWS), :] = ((tile(r) - mu) * scale + b).astype(xs.dtype)


def _kernel(x_hbm, g_hbm, b_hbm, o_hbm, xbuf, gbuf, bbuf, sems, *, HW, rb, wb, wtrig):
    R, C = xbuf.shape
    B = R // HW
    nr, nw = len(rb) - 1, len(wb) - 1

    def rd(k):
        rows = pl.ds(rb[k], rb[k + 1] - rb[k])
        return pltpu.make_async_copy(x_hbm.at[rows], xbuf.at[rows], sems.at[k])

    def wr(k):
        rows = pl.ds(wb[k], wb[k + 1] - wb[k])
        return pltpu.make_async_copy(xbuf.at[rows], o_hbm.at[rows], sems.at[nr + k])

    g_copy = pltpu.make_async_copy(g_hbm, gbuf, sems.at[nr + nw])
    b_copy = pltpu.make_async_copy(b_hbm, bbuf, sems.at[nr + nw + 1])

    rd(0).start()

    def issue(i, carry):
        @pl.when(i == 0)
        def _():
            g_copy.start()
            b_copy.start()

        for k in range(1, nr):
            @pl.when(i == k)
            def _():
                rd(k).start()
        return carry

    jax.lax.fori_loop(0, nr, issue, 0)

    rd(0).wait()
    g_copy.wait()
    b_copy.wait()
    g = gbuf[...].astype(jnp.float32).reshape(1, C)
    b = bbuf[...].astype(jnp.float32).reshape(1, C)

    def body(bi, carry):
        for k in range(1, nr):
            @pl.when(bi == rb[k] // HW)
            def _():
                rd(k).wait()
        for j in range(nw):
            if wtrig[j] < B:
                @pl.when(bi == wtrig[j])
                def _():
                    wr(j).start()
        base = pl.multiple_of(bi * HW, HW)
        _normalize_instance(xbuf.at[pl.ds(base, HW)], g, b)
        return carry

    jax.lax.fori_loop(0, B, body, 0)

    for j in range(nw):
        if wtrig[j] >= B:
            wr(j).start()
    for j in range(nw):
        wr(j).wait()


@jax.jit
def pallas_standalone__instancenorm__sampling_kernel(
    x: jax.Array,
    g: jax.Array,
    b: jax.Array,
):
    B, C, H, W = x.shape
    HW = H * W
    R = B * HW
    xt = jnp.transpose(x, (0, 2, 3, 1)).reshape(R, C)

    half = (B // 2) * HW
    rb = (0, half, R - HW // 2, R)
    wb = (0, half, R)
    wtrig = (B // 2, B)

    out = pl.pallas_call(
        functools.partial(_kernel, HW=HW, rb=rb, wb=wb, wtrig=wtrig),
        in_specs=[pl.BlockSpec(memory_space=pl.ANY)] * 3,
        out_specs=pl.BlockSpec(memory_space=pl.ANY),
        out_shape=jax.ShapeDtypeStruct((R, C), x.dtype),
        scratch_shapes=[
            pltpu.VMEM((R, C), x.dtype),
            pltpu.VMEM((C,), g.dtype),
            pltpu.VMEM((C,), b.dtype),
            pltpu.SemaphoreType.DMA((len(rb) + len(wb),)),
        ],
        compiler_params=pltpu.CompilerParams(
            vmem_limit_bytes=48 * 1024 * 1024,
            disable_semaphore_checks=True,
        ),
    )(xt, g, b)
    return jnp.transpose(out.reshape(B, H, W, C), (0, 3, 1, 2))
```
